```python
import os as _os
_os.environ.setdefault("JAX_PLATFORMS", "cpu")
import jax
import jax.numpy as jnp

def _softmax(x, axis=-1):
    return jax.nn.softmax(x, axis=axis)
def _gelu(x):
    return jax.nn.gelu(x, approximate=True)
def _silu(x):
    return jax.nn.silu(x)
def _sigmoid(x):
    return jax.nn.sigmoid(x)
def _layernorm(x, axis=-1, eps=1e-5):
    m = jnp.mean(x, axis=axis, keepdims=True)
    v = jnp.var(x, axis=axis, keepdims=True)
    return (x - m) / jnp.sqrt(v + eps)
def _scatter_add(tgt, idx, src, axis=0):
    return tgt.at[idx].add(src)
def _segment_sum(src, seg, n):
    return jax.ops.segment_sum(src, seg, n)
class _Rng:
    def __init__(self, key):
        self._k = key
    def _next(self):
        self._k, sub = jax.random.split(self._k)
        return sub
    def normal(self, shape):
        return jax.random.normal(self._next(), shape, dtype=jnp.bfloat16)
    def randint(self, lo, hi, shape):
        return jax.random.randint(self._next(), shape, lo, hi, dtype=jnp.int32)
    def uniform(self, shape, lo=0.0, hi=1.0):
        return jax.random.uniform(self._next(), shape, jnp.bfloat16, lo, hi)
    def permutation(self, n):
        return jax.random.permutation(self._next(), n)


kernel_name = 'interleave_layers__sliding_local_dilated__mixer_s_mlp__prompt'

def setup_inputs():
    _rng = _Rng(jax.random.key(int.from_bytes(__import__("os").urandom(4), "little")))
    _w = (lambda a: (lambda t: t.astype(jnp.bfloat16) if jnp.issubdtype(t.dtype, jnp.floating) else t)(jnp.asarray(a)))
    def _A_setup():
        B, S, D = 1, 2048, 448
        return {
            "x": _w((lambda *s: _rng.normal(s) * 0.05)(B, S, D)),
            "wqkv": _w((lambda *s: _rng.normal(s) * 0.05)(D, 3 * D)),
            "wo": _w((lambda *s: _rng.normal(s) * 0.05)(D, D)),
        }
    _A_in = _A_setup()

    def _B_setup():
        B, S, D, F = 1, 2048, 448, 1792
        return {
            "x":  _w((lambda *s: _rng.normal(s) * 0.05)(B, S, D)),
            "w1": _w((lambda *s: _rng.normal(s) * 0.8)(D, D) * (D ** -0.5)),
            "w2": _w((lambda *s: _rng.normal(s) * 0.8)(D, D) * (D ** -0.5)),
            "w3": _w((lambda *s: _rng.normal(s) * 0.8)(D, F) * (D ** -0.5)),
            "w4": _w((lambda *s: _rng.normal(s) * 0.8)(F, D) * (F ** -0.5)),
        }
    _B_in = _B_setup()

    return {
        "A_x": _A_in["x"],
        "A_wqkv": _A_in["wqkv"],
        "A_wo": _A_in["wo"],
        "B_x": _B_in["x"],
        "B_w1": _B_in["w1"],
        "B_w2": _B_in["w2"],
        "B_w3": _B_in["w3"],
        "B_w4": _B_in["w4"],
    }

def reference(A_x, A_wqkv, A_wo, B_x, B_w1, B_w2, B_w3, B_w4):
    def _A_ref(x, wqkv, wo):
        B, S, D = x.shape
        H = 16; Dh = D // H
        W, dil = 8, 2
        qkv = (lambda x, *d: x.transpose(*d))((x @ wqkv).reshape(B, S, 3, H, Dh), 2, 0, 3, 1, 4)
        q, k, v = qkv[0], qkv[1], qkv[2]
        scale = Dh ** -0.5
        pos = jnp.arange(S)
        off = jnp.arange(W) * dil
        idx = pos[:, None] - off[None, :]
        mask = idx >= 0
        idx_c = jnp.where(mask, idx, 0).reshape(-1)
        kg = k[:, :, idx_c, :].reshape(B, H, S, W, Dh)
        vg = v[:, :, idx_c, :].reshape(B, H, S, W, Dh)
        logits = jnp.einsum("bhsd,bhswd->bhsw", q, kg) * scale
        logits = jnp.where(mask[None, None, :, :], logits, -1e9)
        attn = _softmax(logits, axis=-1)
        o = jnp.einsum("bhsw,bhswd->bhsd", attn, vg)
        return (lambda x, *d: x.transpose(*d))(o, 0, 2, 1, 3).reshape(B, S, D) @ wo

    def _B_ref(x, w1, w2, w3, w4):
        B, S, D = x.shape
        h = _gelu(_layernorm(x, axis=-1) @ w1)
        c = D // 4
        g0 = jnp.pad(h[:, :, 0*c:1*c], ((0, 0), (1, 0), (0, 0)))[:, :S, :]
        g1 = jnp.pad(h[:, :, 1*c:2*c], ((0, 0), (0, 1), (0, 0)))[:, 1:, :]
        g2 = jnp.pad(h[:, :, 2*c:3*c], ((0, 0), (2, 0), (0, 0)))[:, :S, :]
        g3 = jnp.pad(h[:, :, 3*c:   ], ((0, 0), (0, 2), (0, 0)))[:, 2:, :]
        hs = jnp.concatenate([g0, g1, g2, g3], axis=-1) @ w2
        x1 = x + hs
        h2 = _gelu(_layernorm(x1, axis=-1) @ w3) @ w4
        return x1 + h2

    x = A_x
    x = x + _A_ref(_layernorm(x, axis=-1), A_wqkv, A_wo)
    x = x + _B_ref(_layernorm(x, axis=-1), B_w1, B_w2, B_w3, B_w4)
    x = x + _A_ref(_layernorm(x, axis=-1), A_wqkv, A_wo)
    x = x + _B_ref(_layernorm(x, axis=-1), B_w1, B_w2, B_w3, B_w4)
    return x
```

```python
import contextlib
import functools
import math

import jax
import jax.numpy as jnp
from jax import lax
import jax.experimental.pallas as pl
import jax.experimental.pallas.tpu as pltpu

S, D, H, DH, W, F = 2048, 448, 16, 28, 8, 1792
L = 128
T = 2 * L
NB = S // T
NI = 2 * NB
K2 = D // 2
C = D // 4
EPS = 1e-5
BF16, F32, U32 = jnp.bfloat16, jnp.float32, jnp.uint32

_GC0 = 2.0 * math.sqrt(2.0 / math.pi)
_GC1 = 8.0 * 0.044715 * math.sqrt(2.0 / math.pi)
_EXP2_SCALE = DH ** -0.5 * math.log2(math.e)
_MASKED = -1e9 * DH ** 0.5


def _gelu_half(z):
    u = (z * z * _GC1 + _GC0) * z
    return z * jnp.tanh(u) + z


def _words(x):
    return pltpu.bitcast(x, U32)


def _act_combos(b11, b12, b21, b22):
    return b11 + b22, b11, b12 - b22, b21 - b11, b22, b11 + b12, b21 + b22


def _weight_combos(a11, a12, a21, a22):
    return a11 + a22, a21 + a22, a11, a22, a11 + a12, a21 - a11, a12 - a22


HEAD = ("X0 X1 L0 q L1 Q0 W1 S0 V0 P0 Q1 S1 o V1 P1 B0 X2 L2 N0 Q2 S2 1 B1 N1 C0 X3 L3 V2 P2 C1 "
        "W2 H0 2 Q3 3 E0 M0 B2 F0:q,a S3 N2 4 V3 X4 X5 X6 X7 L4 C2 G0:,h H1")
TAIL = "O12 T12 P15 E13 B15 M13 F13 N15 C15 G13 H14 H15 E14 O13 E15 M14 F14 T13 M15 F15 G14 O14 G15 T14 O15 T15"
FIRST = 4


def make_kernel(UNROLL=1, scopes=False, order="P E M Q:q,, S B N V:x,,x O L F C G:,h, H", flags=None, CH=32,
                head=HEAD, tail=TAIL, merge_ln=False, KPV=4, NCH=1, NOCSE=True, KL=2, KM=1, KN=3, KO=0, KH=0, KS=8, only=None, KW=2, KPH=8):

    def kernel(x_hbm, wqkv_hbm, wo_hbm, w1_hbm, w2_hbm, w3_hbm, w4t_hbm, out_hbm,
               xin, wqkv_in, wo_in, w1_in, w2_in, w3_in, w4_in, tmp, tmp_a, tmp_b, tmp_o,
               wqk_t, wv_t, wo_t, w1_t, w2_t, w3_t, w4_t,
               xs, xa_s, y_s, h_s, kp_s, vp_s,
               qk0, qk1, vo0, vo1, hs0, hs1, x10, x11, zero_s, p0, p1,
               y0, y1, o0, o1, z0, z1, h0, h1, s0, s1, g0, g1,
               pa_q, pb_q, pa_v, pb_v, pa_o, pb_o, pa_1, pb_1, pa_2, pb_2, pa_3, pb_3, pa_4, pb_4,
               g_s, stage, sems, osem):
        qk_s, vo_s, hs_s, x1_s = (qk0, qk1), (vo0, vo1), (hs0, hs1), (x10, x11)
        for i in range(3):
            zero_s[i] = 0
        p_s = (p0, p1)
        op_y, op_o, op_z, op_h, op_s, op_g = (y0, y1), (o0, o1), (z0, z1), (h0, h1), (s0, s1), (g0, g1)
        spans = [(0, L), (L, K2), (K2, K2 + L), (K2 + L, D)]
        x_parts = [(0, 2 * T), (2 * T, 4 * T), (4 * T, S)]
        copies = (
            [(wqkv_hbm.at[k0:k1, :], wqkv_in.at[k0:k1, :]) for k0, k1 in spans]
            + [(x_hbm.at[:, s0:s1], xin.at[:, s0:s1]) for s0, s1 in x_parts]
            + [(wo_hbm, wo_in), (w1_hbm, w1_in), (w2_hbm, w2_in), (w3_hbm, w3_in), (w4t_hbm, w4_in.at[0:D, :])])
        dmas = [pltpu.make_async_copy(s, d, sems.at[i]) for i, (s, d) in enumerate(copies)]
        d_qkv, d_x, (d_o, d_1, d_2, d_3, d_4) = dmas[0:4], dmas[4:7], dmas[7:]

        lane = lax.broadcasted_iota(jnp.int32, (1, L), 1)
        lane8 = lax.broadcasted_iota(jnp.int32, (8, L), 1)
        odd = (lane & 1) == 1
        low = lane < L // 2

        def matmul(w_ref, op_ref, pa, pb, fin, gates=((),) * 4):
            m2 = pa.shape[0]
            kk = w_ref.shape[2]
            full = slice(0, m2)

            def prod(i, r=full, k=slice(0, kk)):
                w = pltpu.bitcast(w_ref[i, r.start // 2:r.stop // 2, k], BF16)
                x = pltpu.bitcast(op_ref[i, k.start // 2:k.stop // 2], BF16)
                return jnp.dot(w, x, preferred_element_type=F32)
            a, b = prod(1), prod(3)
            for ref in gates[0]:
                after(ref, a)
            pa[...] = a
            pb[...] = b
            fin(1, 0, full, a + b)
            a, b = prod(2), prod(4)
            for ref in gates[1]:
                after(ref, a)
            pa[...] = a - pa[...]
            pb[...] = pb[...] - b
            fin(0, 1, full, a + b)
            a, b = prod(0), prod(5)
            for ref in gates[2]:
                after(ref, a)
            pb[...] = pb[...] + a
            fin(1, 1, full, pa[...] + a + b)
            if kk == K2:
                for r in (slice(0, m2 // 2), slice(m2 // 2, m2)):
                    fin(0, 0, r, pb[r] + prod(6, r))
            else:
                pb[...] = pb[...] + prod(6, full, slice(0, kk - L))
                for r in (slice(0, 64), slice(64, 128), slice(128, 176), slice(176, 224)):
                    fin(0, 0, r, pb[r] + prod(6, r, slice(kk - L, kk)))

        def at(i, n, r):
            return slice(i * n + r.start, i * n + r.stop)

        def half(i, n):
            return slice(i * n, (i + 1) * n)

        def paced(depth, steps, load, finish):
            ready = []
            for n in range(len(steps) + depth):
                if n < len(steps):
                    ready.append(load(*steps[n]))
                if n >= depth:
                    finish(*steps[n - depth], *ready.pop(0))

        def pack16(x):
            return jnp.concatenate([
                _words(pltpu.pack_elementwise([x[r:r + 8], x[r + 8:r + 16]], packed_dtype=BF16))
                for r in range(0, x.shape[0], 16)], axis=0)

        def total(rows, fn):
            acc = [None] * NCH
            for n, r in enumerate(range(0, D, 8)):
                x = fn(rows(slice(r, r + 8)))
                acc[n % NCH] = x if acc[n % NCH] is None else acc[n % NCH] + x
            return jnp.sum(functools.reduce(jnp.add, acc), axis=0, keepdims=True)

        def stats(ref, i):
            m = total(lambda r: ref[i, r, :], lambda x: x) * (1.0 / D)
            i2 = i + zero_s[1] if NOCSE else i
            v = total(lambda r: ref[i2, r, :], lambda x: (x - m) * (x - m)) * (1.0 / D)
            return m, lax.rsqrt(v + EPS), v

        def put_operands(dst, ref, base, fn=lambda i, x: x, depth=0):
            j = base + zero_s[2] if NOCSE else base

            def load(r):
                return ([ref[j + i, r + kh * K2:r + kh * K2 + 16, :]
                         for kh in range(2) for i in range(2)],)

            def finish(r, x):
                for i, c in enumerate(_act_combos(*[fn(i % 2, v) for i, v in enumerate(x)])):
                    dst[i, r // 2:r // 2 + 8] = pack16(c)
                if depth:
                    after(ref, c)
            paced(depth, [(r,) for r in range(0, K2, 16)], load, finish)

        def after(ref, value):
            ref[ref.shape[0] - 1 + zero_s[0], 0:8, :] = value[0:8]

        def moved_up(prev, cur, s):
            return pltpu.roll(jnp.where(lane >= L - s, prev, cur), s, 1)

        def moved_down(cur, nxt, s):
            return pltpu.roll(jnp.where(lane < s, nxt, cur), L - s, 1)

        def window(prev, cur):
            src = {(t, 0): cur[t] for t in range(2)}
            for t in range(2):
                for s in range(2, 8 + t, 2):
                    src[t, s] = moved_up(prev[t], cur[t], s)
            return [[src[(j - w) % 2, 2 * ((w - j + 1) // 2)] for w in range(W)] for j in range(2)]

        def permute(x, idx):
            return jnp.concatenate(
                [jnp.take_along_axis(x[r:r + 8], idx, axis=1) for r in range(0, x.shape[0], 8)],
                axis=0)

        def st_load(b):
            xw = xin.bitcast(U32)
            u = lane8 & (L // 2 - 1)
            idx = 4 * (u >> 1) + (u & 1)
            j = 2 * (lane8 >> 6)
            g0 = permute(xw[:, b * T:b * T + L], idx + j)
            g1 = permute(xw[:, b * T + L:(b + 1) * T], idx + 2 - j)
            tiles = jnp.where(low, g0, g1), pltpu.roll(jnp.where(low, g1, g0), L // 2, 1)
            for i in range(2):
                xs[2 * b + i] = pltpu.bitcast(tiles[i], BF16).astype(F32)

        def yslot(t):
            return t % 2 if isinstance(t, int) else 0

        def st_ln1(t, k):
            b = t % NB
            st = [stats(xs, 2 * b + i) for i in range(2)]
            put_operands(op_y[yslot(t)], xs, 2 * b, lambda i, x: (x - st[i][0]) * st[i][1], KL)

        def st_qk(t, k, gates):
            def fin(i, j, rr, val):
                qk_s[k][j, at(i, D, rr), :] = val
            matmul(wqk_t, op_y[yslot(t)], pa_q, pb_q, fin, gates)

        def st_v(t, k, gates):
            def fin(i, j, rr, val):
                vo_s[k][j + (zero_s[0] if KPV else 0), at(i, K2, rr), :] = val
            matmul(wv_t, op_y[yslot(t)], pa_v, pb_v, fin, gates)

        d_order = list(range(DH // 2, DH)) + list(range(DH // 2))

        def st_probs(t, k):
            first = (t % NB) == 0
            for hh in range(2):
                acc = [[None] * W, [None] * W]

                def load(d):
                    r0 = d * H + 8 * hh
                    q0 = r0 + d * H
                    return ([qk_s[k][i, q0:q0 + 8, :] for i in range(2)],
                            [qk_s[k][i, q0 + H:q0 + H + 8, :] for i in range(2)],
                            [kp_s[i, r0:r0 + 8, :] for i in range(2)])

                def finish(d, q, cur, prev):
                    r0 = d * H + 8 * hh
                    win = window(prev, cur)
                    for i in range(2):
                        for w in range(W):
                            p = q[i] * win[i][w]
                            acc[i][w] = p if acc[i][w] is None else acc[i][w] + p
                        kp_s[i, r0:r0 + 8, :] = cur[i]
                    if KS:
                        after(qk_s[k], acc[0][W - 1])
                paced(KS, [(d,) for d in d_order], load, finish)
                for i in range(2):
                    logits = []
                    for w in range(W):
                        s = 2 * ((w - i + 1) // 2)
                        a = acc[i][w]
                        if s:
                            a = jnp.where(jnp.logical_and(first, lane < s), _MASKED, a)
                        logits.append(a)
                    m = functools.reduce(jnp.maximum, logits)
                    e = [jnp.exp2((a - m) * _EXP2_SCALE) for a in logits]
                    inv = 1.0 / functools.reduce(jnp.add, e)
                    for w in range(W):
                        p_s[k][hh, i, w] = e[w] * inv

        def st_pv(t, k):
            z = zero_s[0] if KPV else 0
            probs = [[[p_s[k][hh, i, w] for w in range(W)] for i in range(2)] for hh in range(2)]
            steps = [(hh, slice(d * H + 8 * hh, d * H + 8 * hh + 8))
                     for hh in range(2) for d in d_order]
            paced(KPH if isinstance(t, int) else KPV, steps,
                  lambda hh, r: ([vo_s[k][i, r, :] for i in range(2)],
                                 [vp_s[i, r, :] for i in range(2)]),
                  lambda hh, r, cur, prev: pv_step(k, z, r, probs[hh], cur, prev))
            put_operands(op_o[k], vo_s[k], 2, depth=KO)

        def pv_step(k, z, r, p, cur, prev):
            win = window(prev, cur)
            for i in range(2):
                acc = p[i][0] * win[i][0]
                for w in range(1, W):
                    acc = acc + p[i][w] * win[i][w]
                vo_s[k][2 + i + z, r, :] = acc
                vp_s[i, r, :] = cur[i]

        def st_wo(t, k, gates):
            b = t % NB

            def fin(i, j, rr, val):
                r = at(i, K2, rr)
                xa_s[2 * b + j, r, :] = xs[2 * b + j, r, :] + val
            matmul(wo_t, op_o[k], pa_o, pb_o, fin, gates)

        def st_ln23(t, k):
            b = t % NB
            st = []
            for i in range(2):
                m, r, v = stats(xa_s, 2 * b + i)
                y_s[2 * b + i] = (xa_s[2 * b + i + (zero_s[2] if NOCSE else 0)] - m) * r
                st.append(0.5 * lax.rsqrt(v * r * r + EPS))
            if merge_ln:
                return put_operands(op_z[k], y_s, 2 * b, lambda i, x: x * st[i], KN)
            st = [stats(y_s, 2 * b + i) for i in range(2)]
            st = [(m, r * 0.5) for m, r, _ in st]
            put_operands(op_z[k], y_s, 2 * b, lambda i, x: (x - st[i][0]) * st[i][1], KN)

        def st_w1(t, k, gates):
            b = t % NB

            def fin(i, j, rr, val):
                h_s[2 * b + j, at(i, K2, rr), :] = _gelu_half(val)
            matmul(w1_t, op_z[k], pa_1, pb_1, fin, gates)

        def st_shift(t, k):
            b = t % NB
            bl = jnp.maximum(b - 1, 0)
            br = jnp.minimum(b + 1, NB - 1)
            for g in range(4):
                r = half(g, C)
                h0, h1 = h_s[2 * b, r, :], h_s[2 * b + 1, r, :]
                if g % 2 == 0:
                    edge = jnp.where(b > 0, h_s[2 * bl + 1, r, :], 0.0)
                else:
                    edge = jnp.where(b < NB - 1, h_s[2 * br, r, :], 0.0)
                if g == 0:
                    new = (moved_up(edge, jnp.where(odd, h1, h0), 1),
                           jnp.where(odd, pltpu.roll(h1, 1, 1), pltpu.roll(h0, L - 1, 1)))
                elif g == 1:
                    new = (jnp.where(odd, pltpu.roll(h1, 1, 1), pltpu.roll(h0, L - 1, 1)),
                           moved_down(jnp.where(odd, h1, h0), edge, 1))
                elif g == 2:
                    new = moved_up(edge, h1, 2), h0
                else:
                    new = h1, moved_down(h0, edge, 2)
                for j in range(2):
                    hs_s[k][j, r, :] = new[j]
            put_operands(op_h[k], hs_s[k], 0, depth=KH)

        def st_w2(t, k, gates):
            b = t % NB

            def fin(i, j, rr, val):
                r = at(i, K2, rr)
                x1 = y_s[2 * b + j, r, :] + val
                x1_s[k][j, r, :] = x1
                xs[2 * b + j, r, :] = xa_s[2 * b + j, r, :] + x1
            matmul(w2_t, op_h[k], pa_2, pb_2, fin, gates)

        def st_ln4(t, k):
            st = [stats(x1_s[k], i) for i in range(2)]
            st = [(m, r * 0.5) for m, r, _ in st]
            put_operands(op_s[k], x1_s[k], 0, lambda i, x: (x - st[i][0]) * st[i][1], KM)

        def st_w3(t, k, gates):
            def put(i, x, r=slice(0, F // 2)):
                op_g[k][i, r.start // 2:r.stop // 2] = pack16(x)

            def fin(i, j, rr, val):
                g = _gelu_half(val)
                if (i, j) == (1, 0):
                    g_s[0] = g
                elif (i, j) == (0, 1):
                    g_s[1] = g
                elif (i, j) == (1, 1):
                    g_s[2] = g
                    put(4, g)
                    put(2, g_s[1] - g)
                    put(6, g_s[0] + g)
                else:
                    put(1, g, rr)
                    put(3, g_s[0, rr] - g, rr)
                    put(5, g + g_s[1, rr], rr)
                    put(0, g + g_s[2, rr], rr)
            matmul(w3_t, op_s[k], pa_3, pb_3, fin, gates)

        def st_w4(t, k, gates):
            b = t % NB

            def fin(i, j, rr, val):
                r = at(i, K2, rr)
                xs[2 * b + j, r, :] = xs[2 * b + j, r, :] + val
            matmul(w4_t, op_g[k], pa_4, pb_4, fin, gates)

        def st_stage(b):
            t0, t1 = [
                _words(pltpu.pack_elementwise(
                    [xs[2 * b + i, pl.ds(e, K2, stride=2), :] for e in range(2)], packed_dtype=BF16))
                for i in range(2)]
            t1 = pltpu.roll(t1, L // 2, 1)
            idx = 2 * (lane8 >> 2) + (lane8 & 1)
            j = ((lane8 >> 1) & 1) * (L // 2)
            sw = stage.bitcast(U32)
            sw[b, :, 0:L] = permute(jnp.where(low, t0, t1), idx + j)
            sw[b, :, L:T] = permute(jnp.where(low, t1, t0), idx + L // 2 - j)

        def out_copy(b):
            return pltpu.make_async_copy(
                stage.at[b], out_hbm.at[:, pl.ds(pl.multiple_of(b * T, T), T)], osem.at[b])

        def transposed(w):
            return _words(pltpu.bitcast(pack16(w), BF16).T)

        def halves(words):
            return [pltpu.unpack_elementwise(words, index=e, packed_dtype=BF16, unpacked_dtype=F32)
                    for e in range(2)]

        def combine(ref, steps, load, put):
            def finish(step, even, odd):
                for i, pair in enumerate(zip(_weight_combos(*even), _weight_combos(*odd))):
                    w = _words(pltpu.pack_elementwise(list(pair), packed_dtype=BF16))
                    put(step, i, w)
                if KW:
                    ref[pl.ds(pl.multiple_of(ref.shape[0] - 8 + 8 * zero_s[0], 8), 8), 0:L] = w
            paced(KW, [(step,) for step in steps], load, finish)

        def put_tile(dst, r, c, i, w):
            kw = min(L, dst.shape[2] - c * L)
            dst[i, r:r + 8, c * L:c * L + kw] = w[:, 0:kw]

        def prep_qkv():
            n = 3 * D // 2
            for c, (k0, k1) in enumerate(spans):
                d_qkv[c].wait()
                tmp[c * n:(c + 1) * n, 0:k1 - k0] = transposed(wqkv_in[k0:k1, :].astype(F32))
            arrive((), (d_x[1], d_o, d_1, d_2))
            steps = [(wqk_t, t, d, c, (2 * d + t) * 8)
                     for d in range(DH // 2) for t in range(2) for c in range(2)]
            steps += [(wv_t, 2, d, c, d * 8) for d in range(DH // 2) for c in range(2)]

            def load(step):
                _, t, d, c, _ = step
                return [[halves(tmp[pl.ds((c + 2 * kh) * n + (t * D + e * DH + d + mh * DH // 2) // 2,
                                          H // 2, stride=DH), :])[d % 2]
                         for mh in range(2) for kh in range(2)] for e in range(2)]
            combine(tmp, steps, load, lambda step, i, w: put_tile(step[0], step[4], step[3], i, w))

        def prep_t(dst, buf, rows):
            n = 2 * dst.shape[1]
            for c, (k0, k1) in enumerate(spans):
                buf[c * n:(c + 1) * n, 0:k1 - k0] = transposed(rows(k0, k1))

            def load(step):
                r, c = step
                return zip(*[halves(buf[pl.ds((c + 2 * kh) * n + mh * n // 2 + r, 8), :])
                             for mh in range(2) for kh in range(2)])
            combine(buf, [(r, c) for r in range(0, n // 2, 8) for c in range(2)], load,
                    lambda step, i, w: put_tile(dst, *step, i, w))

        def prep_wo():
            for c in range(4):
                kw = min(L, D - c * L)
                tmp_o[c, :, 0:kw] = wo_in[:, c * L:c * L + kw].astype(F32)

            def rows(k0, k1):
                return jnp.concatenate([
                    jnp.concatenate(
                        [tmp_o[c, pl.ds(d, H, stride=DH), :] for d in range(k0 // H, k1 // H)],
                        axis=0)[:, 0:min(L, D - c * L)]
                    for c in range(4)], axis=1)
            prep_t(wo_t, tmp_a, rows)

        def prep_plain(src, dst, buf):
            prep_t(dst, buf, lambda k0, k1: src[k0:k1, :].astype(F32))

        def prep_w4():
            ww = w4_in.bitcast(U32)
            idx = (lane8 & -16) + ((lane8 & 15) >> 1) + 8 * (lane8 & 1)

            def load(step):
                r, c = step
                return zip(*[
                    halves(permute(ww[pl.ds(mh * K2 // 2 + r, 8), pl.ds(kh * F // 2 + c * L, L)], idx))
                    for mh in range(2) for kh in range(2)])
            combine(ww, [(r, c) for c in range(F // 2 // L) for r in range(0, K2 // 2, 8)], load,
                    lambda step, i, w: put_tile(w4_t, *step, i, w))

        def run(ch, t, k, gates=""):
            refs = dict(h=h_s, x=xs, a=xa_s, q=qk_s[k], v=vo_s[k], s=x1_s[k])
            gates = [[refs[g] for g in part] for part in (gates + ",,,").split(",")]
            if ch in "QVBCEFG":
                mm = dict(Q=st_qk, V=st_v, B=st_wo, C=st_w1, E=st_w2, F=st_w3, G=st_w4)[ch]
                mm(t, k, gates)
            elif ch == "X":
                st_load(t)
            elif ch == "O":
                st_stage(t % NB)
            elif ch == "T":
                out_copy(t % NB).start()
            else:
                dict(S=st_probs, P=st_pv, L=st_ln1, N=st_ln23, H=st_shift, M=st_ln4)[ch](t, k)

        def arrive(landed, started):
            for d in landed:
                d.wait()
            for d in started:
                d.start()

        def run_list(prog):
            steps = {
                "q": prep_qkv, "o": prep_wo, "4": prep_w4,
                "1": lambda: prep_plain(w1_in, w1_t, tmp_b),
                "2": lambda: prep_plain(w2_in, w2_t, tmp_a),
                "3": lambda: prep_plain(w3_in, w3_t, tmp),
                "W1": lambda: arrive((d_x[1], d_o, d_1, d_2), (d_3, d_4, d_x[2])),
                "W2": lambda: arrive((d_3, d_4, d_x[2]), ()),
            }
            for word in prog.split():
                if word in steps:
                    steps[word]()
                else:
                    word, _, gates = word.partition(":")
                    t = int(word[1:])
                    run(word[0], t, (t + 1) % 2, gates)

        def scope(name):
            return jax.named_scope(name) if scopes else contextlib.nullcontext()

        with scope("head"):
            arrive((), d_x[0:1] + d_qkv)
            kp_s[...] = jnp.zeros_like(kp_s)
            vp_s[...] = jnp.zeros_like(vp_s)
            arrive(d_x[0:1], ())
            if only in (None, "head"):
                run_list(head)

        lag = dict(L=-1, Q=0, S=0, V=0, P=1, B=1, N=1, C=1, H=2, E=3, M=3, F=3, G=3, O=4 - NB)

        def main(i, carry):
            for j in range(UNROLL):
                t = FIRST + i * UNROLL + j
                for word in order.split():
                    run(word[0], t - lag[word[0]], 0, word[2:])

                @pl.when(t - 4 >= NB)
                def _():
                    run("T", t - 4, 0)
            return carry

        with scope("main"):
            if only in (None, 'main'):
                lax.fori_loop(0, (NI - FIRST) // UNROLL, main, 0)

        if only:
            keep = [pa_q, pb_q, pa_v, pb_v, pa_o, pb_o, pa_1, pb_1, pa_2, pb_2, pa_3, pb_3, pa_4, pb_4,
                    g_s, y0, o0, z0, h0, s0, g0, p0, qk0, vo0, hs0, x10, kp_s, vp_s,
                    wqk_t, wv_t, wo_t, w1_t, w2_t, w3_t, w4_t]
            acc = 0
            for r in keep:
                v = r[...] if r.shape[-1] == L else r[..., 0:L]
                acc = acc + pltpu.bitcast(v.reshape(-1, 8, L), U32).astype(jnp.int32).sum(0)
            xs[0, 0:8, :] = pltpu.bitcast(acc, F32)
            st_stage(0)
        with scope("tail"):
            if only in (None, 'tail'):
                run_list(tail)
            for b in range(NB):
                out_copy(b).wait()

    def call(A_x, A_wqkv, A_wo, B_x, B_w1, B_w2, B_w3, B_w4):
        del B_x
        hbm = pl.BlockSpec(memory_space=pltpu.HBM)

        def wbuf(m, k):
            return pltpu.VMEM((7, m // 4, k // 2), U32)

        def pbuf(m):
            return [pltpu.VMEM((m // 2, L), F32)] * 2

        item = pltpu.VMEM((2, D, L), F32)
        out = pl.pallas_call(
            kernel,
            in_specs=[hbm] * 7,
            out_specs=hbm,
            out_shape=jax.ShapeDtypeStruct((D, S), BF16),
            scratch_shapes=[
                pltpu.VMEM((D, S), BF16),
                pltpu.VMEM((D, 3 * D), BF16),
                pltpu.VMEM((D, D), BF16),
                pltpu.VMEM((D, D), BF16),
                pltpu.VMEM((D, D), BF16),
                pltpu.VMEM((D, F), BF16),
                pltpu.VMEM((D + 16, F), BF16),
                pltpu.VMEM((2 * F + 8, L), U32), *[pltpu.VMEM((2 * D + 8, L), U32)] * 2,
                pltpu.VMEM((4, D, L), F32),
                wbuf(2 * D, D), wbuf(D, D), wbuf(D, D), wbuf(D, D), wbuf(D, D),
                wbuf(F, D), wbuf(D, F),
                *[pltpu.VMEM((2 * NB + 1, D, L), F32)] * 2,
                *[pltpu.VMEM((2 * NB + 1, D, L), F32)] * 2,
                item, item,
                *[pltpu.VMEM((3, 2 * D, L), F32)] * 2,
                *[pltpu.VMEM((5, D, L), F32)] * 2,
                *[pltpu.VMEM((3, D, L), F32)] * 4,
                pltpu.SMEM((3,), jnp.int32),
                *[pltpu.VMEM((2, 2, W, 8, L), F32)] * 2,
                *[pltpu.VMEM((7, K2 // 2, L), U32)] * 10, *[pltpu.VMEM((7, F // 4, L), U32)] * 2,
                *pbuf(2 * D), *pbuf(D), *pbuf(D), *pbuf(D), *pbuf(D), *pbuf(F), *pbuf(D),
                pltpu.VMEM((3, F // 2, L), F32),
                pltpu.VMEM((NB, D, T), BF16),
                pltpu.SemaphoreType.DMA((12,)),
                pltpu.SemaphoreType.DMA((NB,)),
            ],
            compiler_params=pltpu.CompilerParams(
                vmem_limit_bytes=100 * 1024 * 1024, flags=flags),
        )(A_x.reshape(S, D).T, A_wqkv, A_wo, B_w1, B_w2, B_w3, B_w4.T)
        return out.T.reshape(1, S, D)

    return call


@jax.jit
def pallas_interleave_layers__sliding_local_dilated__mixer_s_mlp__prompt_kernel(
        A_x, A_wqkv, A_wo, B_x, B_w1, B_w2, B_w3, B_w4):
    return make_kernel()(A_x, A_wqkv, A_wo, B_x, B_w1, B_w2, B_w3, B_w4)
```

```python
import functools
import math

import jax
import jax.numpy as jnp
import numpy as np
from jax import lax
import jax.experimental.pallas as pl
import jax.experimental.pallas.tpu as pltpu

S, D, H, DH, W, F = 2048, 448, 16, 28, 8, 1792
L = 128
T = 2 * L
NB = S // T
NI = 2 * NB
K2 = D // 2
C = D // 4
EPS = 1e-5
BF16, F32, U32 = jnp.bfloat16, jnp.float32, jnp.uint32

G0 = 2.0 * math.sqrt(2.0 / math.pi)
G1 = 4.0 * 0.044715 * G0
EXP2_SCALE = DH ** -0.5 * math.log2(math.e)
MASKED = -1e9 * DH ** 0.5

HEAD = ("X0 X1 L0 L1 W0 q WV Q0:b v S0 V0 P0 Q1 S1 W1 o 1 V1:,,j X2 L2 P1 B0:,a N0 Q2 B1:,j X3 N1 C0 C1:,,h H0 "
        "W2 2 3 L3 V2 E0 M0 F0:rw S2 P2 Q3:g 4 S3 B2:i X4 L4 N2 V3 C2:,h H1 G0:i X5 X6 X7")
FIRST = 4
STEP = "P E:,,s M Q:q S B N V:,,x L F:,x O C G:h H"
LAG = dict(L=-1, Q=0, S=0, V=0, P=1, B=1, N=1, C=1, H=2, E=3, M=3, F=3, G=3, O=4)
TAIL = ("P15 O12 T12 E13 M13 B15 F13:a N15 C15 H14 H15 E14 M14 E15:,s M15 G13:,,x O13 F14 T13 F15 "
        "G14 O14 T14 G15 Z15 Y15")
AHEAD = dict(M=1, N=2, S=5, P=8, L0=0, L1=0, L2=2, N0=3, N1=3, N2=0, M0=0,
             S0=8, S1=8, P2=6, P15=10, S2=6)


def _gelu(z):
    return z * jnp.tanh((z * z * G1 + G0) * z) + z


def _pack(low, high):
    return pltpu.bitcast(pltpu.pack_elementwise([low, high], packed_dtype=BF16), U32)


def _unpack(words):
    return [pltpu.bitcast(words << 16, F32), pltpu.bitcast(words & np.uint32(0xFFFF0000), F32)]


def _act_terms(b11, b12, b21, b22):
    return b11, b21 - b11, b12 - b22, b22, b11 + b22, b11 + b12, b21 + b22


def _weight_terms(a11, a12, a21, a22):
    return a21 + a22, a22, a11, a11 + a12, a11 + a22, a21 - a11, a12 - a22


def _part(i, n):
    return slice(i * n, (i + 1) * n)


def _within(i, n, rows):
    return slice(i * n + rows.start, i * n + rows.stop)


def _paced(ahead, steps, load, finish):
    ready = []
    for n in range(len(steps) + ahead):
        if n < len(steps):
            ready.append(load(steps[n]))
        if n >= ahead:
            finish(steps[n - ahead], *ready.pop(0))


def _permute(x, idx):
    return jnp.concatenate(
        [jnp.take_along_axis(x[r:r + 8], idx, axis=1) for r in range(0, x.shape[0], 8)], axis=0)


def _kernel(x_hbm, wqkv_hbm, wo_hbm, w1_hbm, w2_hbm, w3_hbm, w4t_hbm, out_hbm,
            x_in, w_in, tmp_q, tmp_a, tmp_b, tmp_o, w_t, xs, xa_s, y_s, h_s, kp_s, vp_s,
            qk_s, vo_s, x1_s, zero_s, p_s, op_y, op_o, op_z, op_h, op_s, op_g, partial,
            g_s, stage, sems, osem):
    wqk_in, wv_in, wo_in, w1_in, w2_in, w3_in, w4_in = w_in
    wqk_t, wv_t, wo_t, w1_t, w2_t, w3_t, w4_t = w_t

    copies = [(x_hbm.at[:, 0:2 * T], x_in[0]), (wqkv_hbm.at[:, 0:2 * D], wqk_in),
              (wqkv_hbm.at[:, 2 * D:3 * D], wv_in), (x_hbm.at[:, 2 * T:4 * T], x_in[1]),
              (wo_hbm, wo_in), (w1_hbm, w1_in), (w2_hbm, w2_in), (w3_hbm, w3_in),
              (w4t_hbm, w4_in), (x_hbm.at[:, 4 * T:S], x_in[2])]
    copies = [pltpu.make_async_copy(src, dst.at[0:D, :], sems.at[i])
              for i, (src, dst) in enumerate(copies)]
    for copy in copies:
        copy.start()

    @pl.loop(0, 3)
    def _(i):
        zero_s[i] = 0

    lane = lax.broadcasted_iota(jnp.int32, (1, L), 1)
    lane8 = lax.broadcasted_iota(jnp.int32, (8, L), 1)
    odd = (lane & 1) == 1
    low = lane < L // 2

    def after(ref, value):
        if ref.dtype == BF16:
            rows = pl.ds(pl.multiple_of(K2 + 8 * zero_s[0], 8), 8)
            ref.bitcast(U32)[rows, 0:L] = pltpu.bitcast(value[0:8], U32)
        else:
            ref[ref.shape[0] - 1 + zero_s[0], 0:8, :] = value[0:8]

    def matmul(n, m, op_ref, fin, gates):
        w_ref, (pa, pb) = w_t[n], partial[n]
        m2, kk = m // 2, w_ref.shape[2]
        full = slice(0, m2)

        def prod(i, r=full, k=slice(0, kk)):
            w = pltpu.bitcast(w_ref[i, r.start // 2:r.stop // 2, k], BF16)
            x = pltpu.bitcast(op_ref[i, k.start // 2:k.stop // 2], BF16)
            return jnp.dot(w, x, preferred_element_type=F32)

        def pair(i):
            a, b = prod(2 * i), prod(2 * i + 1)
            for ref in gates[i]:
                after(ref, a)
            return a, b
        a, b = pair(0)
        pa[full] = a
        pb[full] = b
        fin(1, 0, full, a + b)
        a, b = pair(1)
        pa[full] = a - pa[full]
        pb[full] = pb[full] - b
        fin(0, 1, full, a + b)
        a, b = pair(2)
        pb[full] = pb[full] + a
        fin(1, 1, full, pa[full] + a + b)
        if kk == K2:
            for r in (slice(0, m2 // 2), slice(m2 // 2, m2)):
                fin(0, 0, r, pb[r] + prod(6, r))
        else:
            pb[full] = pb[full] + prod(6, full, slice(0, kk - L))
            for r in (slice(0, 64), slice(64, 128), slice(128, 176), slice(176, 224)):
                fin(0, 0, r, pb[r] + prod(6, r, slice(kk - L, kk)))

    def total(ref, i, fn):
        acc = fn(ref[i, 0:8, :])
        for r in range(8, D, 8):
            acc = acc + fn(ref[i, r:r + 8, :])
        return jnp.sum(acc, axis=0, keepdims=True)

    def stats(ref, i):
        m = total(ref, i, lambda x: x) * (1.0 / D)
        i = i if isinstance(i, int) else i + zero_s[1]
        v = total(ref, i, lambda x: (x - m) * (x - m)) * (1.0 / D)
        return m, lax.rsqrt(v + EPS)

    def put_terms(dst, rows_of, ahead=0, ref=None):
        def load(r):
            return [[x for kh in range(2) for x in rows_of(r + kh * K2 + e)] for e in range(2)]

        def finish(r, *rows):
            terms = [_act_terms(*[x() for x in blocks]) for blocks in rows]
            for i, both in enumerate(zip(*terms)):
                dst[i, r // 2:r // 2 + 8] = _pack(*both)
            if ahead:
                after(ref, both[1])
        _paced(ahead, range(0, K2, 16), load, finish)

    def put_operands(dst, ref, base, fn=lambda i, x: x, ahead=0):
        base = base if isinstance(base, int) and not ahead else base + zero_s[2]
        put_terms(dst, lambda r: [functools.partial(fn, i, ref[base + i, pl.ds(r, 8, stride=2), :])
                                  for i in range(2)], ahead, ref)

    def put_norm(dst, ref, base, scale, ahead, shift=0):
        st = [stats(ref, base + i + shift) for i in range(2)]
        if scale != 1.0:
            st = [(m, r * scale) for m, r in st]
        put_operands(dst, ref, base, lambda i, x: (x - st[i][0]) * st[i][1], ahead)

    def moved_up(prev, cur, s):
        return pltpu.roll(jnp.where(lane >= L - s, prev, cur), s, 1)

    def moved_down(cur, nxt, s):
        return pltpu.roll(jnp.where(lane < s, nxt, cur), L - s, 1)

    def window(prev, cur):
        src = {(j, 0): cur[j] for j in range(2)}
        for j in range(2):
            for s in range(2, 8 + j, 2):
                src[j, s] = moved_up(prev[j], cur[j], s)
        return [[src[(j - w) % 2, 2 * ((w - j + 1) // 2)] for w in range(W)] for j in range(2)]

    def st_load(b):
        words = x_in[min(b // 2, 2)].bitcast(U32)
        c = (b - 2 * min(b // 2, 2)) * T
        u = lane8 & (L // 2 - 1)
        idx = 4 * (u >> 1) + (u & 1)
        j = 2 * (lane8 >> 6)
        for r in range(0, K2, 8):
            g0 = _permute(words[r:r + 8, c:c + L], idx + j)
            g1 = _permute(words[r:r + 8, c + L:c + T], idx + 2 - j)
            tiles = jnp.where(low, g0, g1), pltpu.roll(jnp.where(low, g1, g0), L // 2, 1)
            for i in range(2):
                for e, x in enumerate(_unpack(tiles[i])):
                    xs[2 * b + i, pl.ds(2 * r + e, 8, stride=2), :] = x

    def st_qk(b, k, ky, gates):
        def fin(i, j, rows, val):
            qk_s[k][j, _within(i, D, rows), :] = val
        matmul(0, 2 * D, op_y[ky], fin, gates)

    def st_v(b, k, ky, gates):
        def fin(i, j, rows, val):
            vo_s[k][j, _within(i, K2, rows), :] = val
        matmul(1, D, op_y[ky], fin, gates)

    d_order = list(range(DH // 2, DH)) + list(range(DH // 2))

    def st_softmax(b, k, ahead):
        for hh in range(2):
            acc = [[None] * W, [None] * W]

            def load(d):
                r = d * H + 8 * hh
                q = r + d * H
                return ([qk_s[k][i, q:q + 8, :] for i in range(2)],
                        [qk_s[k][i, q + H:q + H + 8, :] for i in range(2)],
                        [kp_s[i, r:r + 8, :] for i in range(2)])

            def finish(d, q, cur, prev):
                r = d * H + 8 * hh
                win = window(prev, cur)
                for i in range(2):
                    for w in range(W):
                        p = q[i] * win[i][w]
                        acc[i][w] = p if acc[i][w] is None else acc[i][w] + p
                    kp_s[i, r:r + 8, :] = cur[i]
                if ahead:
                    after(qk_s[k], acc[0][W - 1])
            _paced(ahead, d_order, load, finish)
            for i in range(2):
                logits = []
                for w in range(W):
                    s = 2 * ((w - i + 1) // 2)
                    logits.append(jnp.where(jnp.logical_and(b == 0, lane < s), MASKED, acc[i][w])
                                  if s else acc[i][w])
                m = functools.reduce(jnp.maximum, logits)
                e = [jnp.exp2((a - m) * EXP2_SCALE) for a in logits]
                inv = 1.0 / functools.reduce(jnp.add, e)
                for w in range(W):
                    p_s[k][2 * hh + i, _part(w, 8)] = e[w] * inv

    def st_mix(b, k, ahead):
        z = zero_s[0]
        probs = [[p_s[k][n, _part(w, 8)] for w in range(W)] for n in range(4)]

        def load(step):
            return ([vo_s[k][i, step[1], :] for i in range(2)],
                    [vp_s[i, step[1], :] for i in range(2)])

        def finish(step, cur, prev):
            hh, r = step
            win = window(prev, cur)
            for i in range(2):
                p = probs[2 * hh + i]
                acc = p[0] * win[i][0]
                for w in range(1, W):
                    acc = acc + p[w] * win[i][w]
                vo_s[k][2 + i + z, r, :] = acc
                vp_s[i, r, :] = cur[i]
        _paced(ahead, [(hh, _part(2 * d + hh, 8)) for hh in range(2) for d in d_order],
               load, finish)

    def st_wo(b, k, ky, gates):
        def fin(i, j, rows, val):
            r = _within(i, K2, rows)
            xa_s[2 * b + j, r, :] = xs[2 * b + j, r, :] + val
        matmul(2, D, op_o[k], fin, gates)

    def st_norm2(b, k, ahead):
        for i in range(2):
            m, r = stats(xa_s, 2 * b + i)
            y_s[2 * b + i, 0:D] = (xa_s[2 * b + i, 0:D] - m) * r
        put_norm(op_z[k], y_s, 2 * b, 0.5, ahead)

    def st_w1(b, k, ky, gates):
        def fin(i, j, rows, val):
            h_s[2 * b + j, _within(i, K2, rows), :] = _gelu(val)
        matmul(3, D, op_z[k], fin, gates)

    def st_shift(b, k):
        before = 2 * jnp.maximum(b - 1, 0) + 1
        behind = 2 * jnp.minimum(b + 1, NB - 1)

        def rows_of(first):
            g, r = first // C, pl.ds(first, 8, stride=2)
            h0, h1 = h_s[2 * b, r, :], h_s[2 * b + 1, r, :]
            if g % 2 == 0:
                edge = jnp.where(b > 0, h_s[before, r, :], 0.0)
            else:
                edge = jnp.where(b < NB - 1, h_s[behind, r, :], 0.0)
            if g < 2:
                inner = jnp.where(odd, pltpu.roll(h1, 1, 1), pltpu.roll(h0, L - 1, 1))
                outer = jnp.where(odd, h1, h0)
            if g == 0:
                new = moved_up(edge, outer, 1), inner
            elif g == 1:
                new = inner, moved_down(outer, edge, 1)
            elif g == 2:
                new = moved_up(edge, h1, 2), h0
            else:
                new = h1, moved_down(h0, edge, 2)
            return [lambda x=x: x for x in new]
        put_terms(op_h[k], rows_of)

    def x1_of(b):
        return x1_s[(b + 1) % 3 if isinstance(b, int) else 0]

    def st_w2(b, k, ky, gates):
        def fin(i, j, rows, val):
            r = _within(i, K2, rows)
            x1_of(b)[j, r, :] = y_s[2 * b + j, r, :] + val
        matmul(4, D, op_h[k], fin, gates)

    def st_w3(b, k, ky, gates):
        def put(i, rows, x):
            op_g[k][i, rows.start // 2:rows.stop // 2] = jnp.concatenate(
                [_pack(x[r:r + 8], x[r + 8:r + 16]) for r in range(0, x.shape[0], 16)], axis=0)

        def fin(i, j, rows, val):
            g = _gelu(val)
            if (i, j) == (1, 0):
                g_s[0, rows] = g
            elif (i, j) == (0, 1):
                g_s[1, rows] = g
            elif (i, j) == (1, 1):
                g_s[2, rows] = g
                put(3, rows, g)
                put(2, rows, g_s[1, rows] - g)
                put(6, rows, g_s[0, rows] + g)
            else:
                put(0, rows, g)
                put(1, rows, g_s[0, rows] - g)
                put(5, rows, g + g_s[1, rows])
                put(4, rows, g + g_s[2, rows])
        matmul(5, F, op_s[k], fin, gates)

    def st_w4(b, k, ky, gates):
        def fin(i, j, rows, val):
            r = _within(i, K2, rows)
            xs[2 * b + j, r, :] = xa_s[2 * b + j, r, :] + x1_of(b)[j, r, :] + val
        matmul(6, D, op_g[k], fin, gates)

    def st_store(b, p):
        idx = 2 * (lane8 >> 2) + (lane8 & 1)
        j = ((lane8 >> 1) & 1) * (L // 2)
        words = stage.bitcast(U32)
        t0, t1 = [_pack(*[xs[2 * b + i, pl.ds(p * K2 + e, K2 // 2, stride=2), :] for e in range(2)])
                  for i in range(2)]
        t1 = pltpu.roll(t1, L // 2, 1)
        words[b, _part(p, K2 // 2), 0:L] = _permute(jnp.where(low, t0, t1), idx + j)
        words[b, _part(p, K2 // 2), L:T] = _permute(jnp.where(low, t1, t0), idx + L // 2 - j)

    def out_copy(b, p):
        start = b * T if isinstance(b, int) else pl.multiple_of(b * T, T)
        return pltpu.make_async_copy(
            stage.at[b, _part(p, K2), :], out_hbm.at[_part(p, K2), pl.ds(start, T)],
            osem.at[2 * b + p])

    spans = [(0, L), (L, K2), (K2, K2 + L), (K2 + L, D)]
    width = [k1 - k0 for k0, k1 in spans]

    def terms(even, odd):
        return [_pack(*both) for both in zip(_weight_terms(*even), _weight_terms(*odd))]

    def transpose_into(buf, n, load):
        for m in range(0, 2 * n, L):
            for c in range(4):
                x = load(*spans[c], slice(m, min(m + L, 2 * n)))
                buf[c * n + m // 2:c * n + (m + x.shape[1]) // 2, 0:width[c]] = pltpu.bitcast(x.T, U32)

    def prep_heads(src, dst, buf):
        n = src.shape[1] // 2
        parts = 2 * n // D
        transpose_into(buf, n, lambda k0, k1, m: src[k0:k1, m])
        for d in range(0, DH // 2, 2):
            for t in range(parts):
                for c in range(2):
                    heads = [[jnp.concatenate(_unpack(buf[pl.ds(
                        (c + 2 * kh) * n + (t * D + e * DH + d + mh * DH // 2) // 2,
                        H // 2, stride=DH), :][:, 0:width[c]]), axis=0)
                        for mh in range(2) for kh in range(2)] for e in range(2)]
                    for i, w in enumerate(terms(*heads)):
                        for e in range(2):
                            dst[i, _part(parts * (d + e) + t, 8), c * L:c * L + width[c]] = w[_part(e, 8)]

    def prep_square(dst, buf, load):
        transpose_into(buf, K2, load)
        for r in range(0, K2 // 2, 8):
            for c in range(2):
                blocks = [_unpack(buf[pl.ds((c + 2 * kh) * K2 + mh * K2 // 2 + r, 8), 0:width[c]])
                          for mh in range(2) for kh in range(2)]
                for i, w in enumerate(terms(*zip(*blocks))):
                    dst[i, r:r + 8, c * L:c * L + width[c]] = w

    def prep_wo():
        for c in range(0, D, L):
            tmp_o[c // L, 0:D, 0:min(L, D - c)] = wo_in[0:D, c:min(c + L, D)].astype(F32)
        prep_square(wo_t, tmp_a, lambda k0, k1, m: jnp.concatenate(
            [tmp_o[m.start // L, pl.ds(d, H, stride=DH), :][:, 0:m.stop - m.start]
             for d in range(k0 // H, k1 // H)], axis=0).astype(BF16))

    def prep_w3():
        for m in range(0, F // 2, L):
            blocks = [w3_in[_part(kh, K2), pl.ds(mh * F // 2 + m, L)].astype(F32)
                      for mh in range(2) for kh in range(2)]
            for i, w in enumerate(_weight_terms(*blocks)):
                w3_t[i, m // 2:(m + L) // 2, :] = pltpu.bitcast(w.astype(BF16).T, U32)

    def prep_w4():
        words = w4_in.bitcast(U32)
        idx = (lane8 & -16) + ((lane8 & 15) >> 1) + 8 * (lane8 & 1)
        for c in range(0, F // 2, L):
            for r in range(0, K2 // 2, 8):
                blocks = [_unpack(_permute(
                    words[pl.ds(mh * K2 // 2 + r, 8), pl.ds(kh * F // 2 + c, L)], idx))
                    for mh in range(2) for kh in range(2)]
                for i, w in enumerate(terms(*zip(*blocks))):
                    w4_t[i, r:r + 8, c:c + L] = w

    def wait(lo, hi):
        for copy in copies[lo:hi]:
            copy.wait()

    setup = {
        "q": lambda: prep_heads(wqk_in, wqk_t, tmp_q), "v": lambda: prep_heads(wv_in, wv_t, tmp_b),
        "1": lambda: prep_square(w1_t, tmp_b, lambda k0, k1, m: w1_in[k0:k1, m]),
        "2": lambda: prep_square(w2_t, tmp_a, lambda k0, k1, m: w2_in[k0:k1, m]),
        "o": prep_wo, "3": prep_w3, "4": prep_w4,
        "W0": lambda: wait(1, 2), "WV": lambda: wait(2, 3), "W1": lambda: wait(3, 6),
        "W2": lambda: wait(6, 10)}
    gated = dict(x=xs, a=xa_s, h=h_s, q=qk_s[0], r=qk_s[1], w=vo_s[1],
                 i=x_in[2], j=x_in[1], b=wv_in, g=w4_in)
    matmuls = dict(Q=st_qk, V=st_v, B=st_wo, C=st_w1, E=st_w2, F=st_w3, G=st_w4)

    def run(name, t, k, ky, gates="", ahead=0):
        b = t % NB
        if name in matmuls:
            gates = [[x1_of(b) if g == "s" else gated[g] for g in part]
                     for part in (gates + ",,").split(",")]
            matmuls[name](b, k, ky, gates)
        elif name == "X":
            st_load(b)
        elif name == "L":
            put_norm(op_y[ky], xs, 2 * b, 1.0, ahead)
        elif name == "S":
            st_softmax(b, k, ahead)
        elif name == "P":
            st_mix(b, k, ahead)
            put_operands(op_o[k], vo_s[k], 2)
        elif name == "N":
            st_norm2(b, k, ahead)
        elif name == "H":
            st_shift(b, k)
        elif name == "M":
            put_norm(op_s[k], x1_of(b), 0, 0.5, ahead, 0 if isinstance(t, int) else zero_s[0])
        else:
            halves = dict(O=(0, 1), T=(0, 1), Y=(0,), Z=(1,))[name]
            for p in halves if name != "T" else ():
                st_store(b, p)
            for p in halves if name != "O" else ():
                out_copy(b, p).start()

    def run_all(program):
        for word in program.split():
            if word in setup:
                setup[word]()
            else:
                word, _, gates = word.partition(":")
                t = int(word[1:])
                run(word[0], t, (t + 1) % 2, t % 2, gates, AHEAD.get(word, AHEAD.get(word[0], 0)))

    kp_s[...] = jnp.zeros_like(kp_s)
    vp_s[...] = jnp.zeros_like(vp_s)
    wait(0, 1)
    run_all(HEAD)

    @pl.loop(FIRST, NI)
    def _(t):
        for word in STEP.split():
            run(word[0], t - LAG[word[0]], 0, 0, word[2:], AHEAD.get(word[0], 0))

        @pl.when(t - LAG["O"] >= NB)
        def _():
            run("T", t - LAG["O"], 0, 0)

    run_all(TAIL)
    for b in range(NB):
        for p in range(2):
            out_copy(b, p).wait()


@jax.jit
def pallas_interleave_layers__sliding_local_dilated__mixer_s_mlp__prompt_kernel(
    A_x: jax.Array,
    A_wqkv: jax.Array,
    A_wo: jax.Array,
    B_x: jax.Array,
    B_w1: jax.Array,
    B_w2: jax.Array,
    B_w3: jax.Array,
    B_w4: jax.Array,
):
    del B_x
    vmem = pltpu.VMEM
    rows = D + 32
    shapes = ((2 * D, D), (D, D), (D, D), (D, D), (D, D), (F, D), (D, F))
    hbm = pl.BlockSpec(memory_space=pltpu.HBM)
    out = pl.pallas_call(
        _kernel,
        in_specs=[hbm] * 7,
        out_specs=hbm,
        out_shape=jax.ShapeDtypeStruct((D, S), BF16),
        scratch_shapes=[
            [vmem((D + 16, n), BF16) for n in (2 * T, 2 * T, 4 * T)],
            [vmem((D + 16, n), BF16) for n in (2 * D, D, D, D, D, F, F)],
            vmem((4 * D + 48, L), U32),
            vmem((2 * D + 32, L), U32), vmem((2 * D + 32, L), U32),
            vmem((4, rows, L), F32),
            [vmem((7, m // 4, k // 2), U32) for m, k in shapes],
            *[vmem((2 * NB + 1, rows, L), F32)] * 4,
            vmem((2, D, L), F32), vmem((2, D, L), F32),
            [vmem((3, 2 * D, L), F32)] * 2,
            [vmem((5, rows, L), F32)] * 2,
            [vmem((3, rows, L), F32)] * 3,
            pltpu.SMEM((3,), jnp.int32),
            [vmem((4, 8 * W, L), F32)] * 2,
            *[[vmem((7, K2 // 2, L), U32)] * 2] * 5,
            [vmem((7, F // 4, L), U32)] * 2,
            [[vmem((m // 2, L), F32)] * 2 for m, _ in shapes],
            vmem((3, F // 2, L), F32),
            vmem((NB, D, T), BF16),
            pltpu.SemaphoreType.DMA((10,)),
            pltpu.SemaphoreType.DMA((2 * NB,)),
        ],
        compiler_params=pltpu.CompilerParams(vmem_limit_bytes=100 * 1024 * 1024),
    )(A_x.reshape(S, D).T, A_wqkv, A_wo, B_w1, B_w2, B_w3, B_w4.T)
    return out.T.reshape(1, S, D)
```
